```python
import jax
import jax.numpy as jnp

def _softmax(x, axis=-1):
    return jax.nn.softmax(x, axis=axis)
def _gelu(x):
    return jax.nn.gelu(x, approximate=True)
def _silu(x):
    return jax.nn.silu(x)
def _sigmoid(x):
    return jax.nn.sigmoid(x)
def _layernorm(x, axis=-1, eps=1e-5):
    m = jnp.mean(x, axis=axis, keepdims=True)
    v = jnp.var(x, axis=axis, keepdims=True)
    return (x - m) / jnp.sqrt(v + eps)
def _scatter_add(tgt, idx, src, axis=0):
    return tgt.at[idx].add(src)
def _segment_sum(src, seg, n):
    return jax.ops.segment_sum(src, seg, n)
class _Rng:
    def __init__(self, key):
        self._k = key
    def _next(self):
        self._k, sub = jax.random.split(self._k)
        return sub
    def normal(self, shape):
        return jax.random.normal(self._next(), shape, dtype=jnp.bfloat16)
    def randint(self, lo, hi, shape):
        return jax.random.randint(self._next(), shape, lo, hi, dtype=jnp.int32)
    def uniform(self, shape, lo=0.0, hi=1.0):
        return jax.random.uniform(self._next(), shape, jnp.bfloat16, lo, hi)
    def permutation(self, n):
        return jax.random.permutation(self._next(), n)


kernel_name = 'gated_mix__compressed_kv_cla__moe_arch_mod__prompt'

def setup_inputs():
    _rng = _Rng(jax.random.key(int.from_bytes(__import__("os").urandom(4), "little")))
    _w = (lambda a: (lambda t: t.astype(jnp.bfloat16) if jnp.issubdtype(t.dtype, jnp.floating) else t)(jnp.asarray(a)))
    def _A_setup():
        B, H, Sq, Sk, D, M = 1, 16, 2048, 2048, 256, 448
        Dc = 4 * D
        return {
            "x": _w((lambda *s: _rng.normal(s) * 0.05)(B, Sq, M)),
            "c_kv": _w((lambda *s: _rng.normal(s) * 0.05)(B, Sk, Dc)),
            "w_q": _w((lambda *s: _rng.normal(s) * 0.05)(M, H, D) * (M ** -0.5)),
            "w_uk": _w((lambda *s: _rng.normal(s) * 0.05)(Dc, H, D) * (Dc ** -0.5)),
            "w_uv": _w((lambda *s: _rng.normal(s) * 0.05)(Dc, H, D) * (Dc ** -0.5)),
            "w_o": _w((lambda *s: _rng.normal(s) * 0.05)(H, D, M) * ((H * D) ** -0.5)),
        }
    _A_in = _A_setup()

    def _B_setup():
        B, S, D, F, C = 1, 2048, 448, 1792, 2
        return {
            "x": _w((lambda *s: _rng.normal(s) * 0.05)(B, S, D)),
            "w_r": _w((lambda *s: _rng.normal(s) * 0.05)(D)),
            "w_gate": _w((lambda *s: _rng.normal(s) * 0.05)(D, F)),
            "w_up": _w((lambda *s: _rng.normal(s) * 0.05)(D, F)),
            "w_down": _w((lambda *s: _rng.normal(s) * 0.05)(F, D)),
        }
    _B_in = _B_setup()

    return {
        "A_x": _A_in["x"],
        "A_c_kv": _A_in["c_kv"],
        "A_w_q": _A_in["w_q"],
        "A_w_uk": _A_in["w_uk"],
        "A_w_uv": _A_in["w_uv"],
        "A_w_o": _A_in["w_o"],
        "B_x": _B_in["x"],
        "B_w_r": _B_in["w_r"],
        "B_w_gate": _B_in["w_gate"],
        "B_w_up": _B_in["w_up"],
        "B_w_down": _B_in["w_down"],
        "gate_w": _w((lambda *s: _rng.normal(s) * 0.05)(448)),
    }

def reference(A_x, A_c_kv, A_w_q, A_w_uk, A_w_uv, A_w_o, B_x, B_w_r, B_w_gate, B_w_up, B_w_down, gate_w):
    def _A_ref(x, c_kv, w_q, w_uk, w_uv, w_o):
        B, Sq, M = x.shape[0], x.shape[1], x.shape[2]
        Sk = c_kv.shape[1]
        H, D = w_q.shape[1], w_q.shape[2]
        q = jnp.einsum("bqm,mhd->bhqd", x, w_q)
        k = jnp.einsum("bkc,chd->bhkd", c_kv, w_uk)
        v = jnp.einsum("bkc,chd->bhkd", c_kv, w_uv)
        scores = jnp.einsum("bhqd,bhkd->bhqk", q, k) * (D ** -0.5)
        off = Sk - Sq
        qi = jnp.arange(Sq)[:, None]
        kj = jnp.arange(Sk)[None, :]
        cmask = kj <= (qi + off)
        scores = jnp.where(cmask[None, None], scores, -1e9)
        p = _softmax(scores, axis=-1)
        ctx = jnp.einsum("bhqk,bhkd->bhqd", p, v)
        return jnp.einsum("bhqd,hdm->bqm", ctx, w_o)

    def _B_ref(x, w_r, w_gate, w_up, w_down):
        B, S, D = x.shape
        C = 2
        r = x @ w_r
        idx = jnp.argsort(-r, axis=-1)[:, :C]
        idx_e = jnp.repeat(idx.reshape(B, C, 1), D, axis=2)
        x_sel = jnp.take_along_axis(x, idx_e, axis=1)
        g = _silu(x_sel @ w_gate)
        u = x_sel @ w_up
        y = (g * u) @ w_down
        r_sel = _sigmoid(jnp.take_along_axis(r, idx, axis=1))
        y = y * r_sel.reshape(B, C, 1)
        b_off = (jnp.arange(B) * S).reshape(B, 1)
        flat_idx = (idx + b_off).reshape(B * C)
        zero = (x * 0.0).reshape(B * S, D)
        upd = _scatter_add(zero, flat_idx, y.reshape(B * C, D), axis=0)
        return x + upd.reshape(B, S, D)

    x = A_x
    g = _sigmoid((x * gate_w).sum(-1, keepdims=True))
    a = _A_ref(x, A_c_kv, A_w_q, A_w_uk, A_w_uv, A_w_o)
    b = _B_ref(x, B_w_r, B_w_gate, B_w_up, B_w_down)
    return g * a + (1 - g) * b
```

```python
import functools
import jax
import jax.numpy as jnp
from jax import lax
from jax.experimental import pallas as pl
from jax.experimental.pallas import tpu as pltpu

S = 2048
M = 448
DC = 1024
H = 16
D = 256
F = 1792
FT = 128
NF = F // FT
TQ = 256
NQ = S // TQ
SUB = TQ // 128
LOG2E = 1.4426950408889634
QSCALE = (D ** -0.5) * LOG2E
NEG = -1e9 * LOG2E
BF = jnp.bfloat16
F32 = jnp.float32
U32 = jnp.uint32

NT = (((1,), (1,)), ((), ()))
NN = (((1,), (0,)), ((), ()))
_dot = functools.partial(lax.dot_general, preferred_element_type=F32)


def _pk(x):
    return pltpu.bitcast(x, U32)


def _up(x):
    return pltpu.bitcast(x, BF)


def _rows(start, n):
    return pl.ds(start // 2, n // 2)


def _head_of_pair(w32, parity):
    if isinstance(parity, int):
        bits = (w32 << 16) if parity == 0 else (w32 & jnp.uint32(0xFFFF0000))
    else:
        sh = (16 - 16 * parity).astype(U32)
        bits = lax.shift_left(w32, jnp.broadcast_to(sh, w32.shape)) & jnp.uint32(0xFFFF0000)
    return pltpu.bitcast(bits, F32)


def _kernel(xT_hbm, c_hbm, wq_hbm, wk_hbm, wv_hbm, woT_hbm, wr_ref, gw_ref,
            wg_hbm, wu_hbm, wdT_hbm, oT_hbm,
            xT, c, wq32, wk32, wv32, woT, wg, wu, wdT, wqT, wkb, wvT, qT, k_s, vT, acc, obuf,
            xsel, y_s, sel_s, g_s, wsem, csem, xsem, msem, osem):

    def wq_copy(p, sl):
        return pltpu.make_async_copy(wq_hbm.bitcast(U32).at[:, p, :], wq32.at[sl], wsem.at[sl, 0])

    def wk_copy(p, sl):
        return pltpu.make_async_copy(wk_hbm.bitcast(U32).at[:, p, :], wk32.at[sl], wsem.at[sl, 1])

    def wv_copy(p, sl):
        return pltpu.make_async_copy(wv_hbm.bitcast(U32).at[:, p, :], wv32.at[sl], wsem.at[sl, 2])

    def c_copy(i):
        r = pl.ds(i * (TQ // 2), TQ // 2)
        return pltpu.make_async_copy(c_hbm.bitcast(U32).at[r, :], c.at[r, :], csem.at[i])

    XW = 512
    def x_copy(i):
        r = pl.ds(i * XW, XW)
        return pltpu.make_async_copy(xT_hbm.bitcast(U32).at[:, r], xT.at[:, r], xsem.at[i])

    def side_copies(first):
        hs = pl.ds(0, 1) if first else pl.ds(1, H - 1)
        cs = pl.ds(0, FT) if first else pl.ds(FT, F - FT)
        o = 0 if first else 4
        return [pltpu.make_async_copy(woT_hbm.bitcast(U32).at[hs], woT.at[hs], msem.at[o]),
                pltpu.make_async_copy(wg_hbm.bitcast(U32).at[:, cs], wg.at[:, cs], msem.at[o + 1]),
                pltpu.make_async_copy(wu_hbm.bitcast(U32).at[:, cs], wu.at[:, cs], msem.at[o + 2]),
                pltpu.make_async_copy(wdT_hbm.bitcast(U32).at[:, cs], wdT.at[:, cs], msem.at[o + 3])]

    def o_copy(i):
        r = pl.ds(i * TQ, TQ)
        return pltpu.make_async_copy(obuf.at[:, r], oT_hbm.bitcast(U32).at[:, r], osem.at[i])

    def prep_k(sl, parity, r0, n):
        wkb[_rows(r0, n), :] = _pk(_head_of_pair(wk32[sl, pl.ds(r0, n), :], parity).astype(BF))

    def prep_v(sl, parity, r0, n):
        wvT[:, pl.ds(r0, n)] = _pk(_head_of_pair(wv32[sl, pl.ds(r0, n), :], parity).T.astype(BF))

    def prep_q(sl, parity, r0, n):
        wqT[:, pl.ds(r0, n)] = _pk(_head_of_pair(wq32[sl, pl.ds(r0, n), :], parity).T.astype(BF))

    def prep_all(sl, parity):
        for j in range(DC // 128):
            prep_k(sl, parity, 128 * j, 128)
        for j in range(4):
            prep_q(sl, parity, 128 * j, min(128, M - 128 * j))
        for j in range(DC // 128):
            prep_v(sl, parity, 128 * j, 128)

    def projk(r0):
        k_s[_rows(r0, TQ), :] = _pk(_dot(_up(c[_rows(r0, TQ), :]), _up(wkb[...]), NN).astype(BF))

    def projq(r0, n=TQ):
        r = pl.ds(r0, n)
        qT[:, r] = _pk((_dot(_up(wqT[...]), _up(xT[:, r]), NN) * QSCALE).astype(BF))

    def projv(r0):
        vT[:, pl.ds(r0, TQ)] = _pk(_dot(_up(wvT[...]), _up(c[_rows(r0, TQ), :]), NT).astype(BF))

    def scores(i):
        tri = (lax.broadcasted_iota(jnp.int32, (128, 128), 0)
               <= lax.broadcasted_iota(jnp.int32, (128, 128), 1))
        base = i * TQ
        q = _up(qT[:, pl.ds(base, TQ)])
        out = []
        for j in range(base // 128 + SUB):
            k0 = 128 * j
            t0 = max(0, j - base // 128)
            s = _dot(_up(k_s[_rows(k0, 128), :]), q[:, 128 * t0:], NN)
            if k0 >= base:
                blk = jnp.where(tri, s[:, 0:128], NEG)
                s = jnp.concatenate([blk, s[:, 128:]], axis=1) if SUB - t0 > 1 else blk
            m = jnp.max(s, axis=0, keepdims=True)
            e = jnp.exp2(s - m)
            out.append((t0, m, jnp.sum(e, axis=0, keepdims=True), e.astype(BF)))
        return out

    def context(chunks):
        scale = [[None] * SUB for _ in chunks]
        for t in range(SUB):
            js = [j for j, ch in enumerate(chunks) if ch[0] <= t]
            col = lambda x, j: x[:, 128 * (t - chunks[j][0]):128 * (t - chunks[j][0] + 1)]
            ms = [col(chunks[j][1], j) for j in js]
            m = functools.reduce(jnp.maximum, ms)
            al = [jnp.exp2(mj - m) for mj in ms]
            l = functools.reduce(jnp.add, [a * col(chunks[j][2], j) for a, j in zip(al, js)])
            li = 1.0 / l
            for a, j in zip(al, js):
                scale[j][t] = a * li
        ctx = [None] * SUB
        for j, (t0, _, _, p) in enumerate(chunks):
            rr = _dot(_up(vT[:, pl.ds(128 * j, 128)]), p, NN)
            for t in range(t0, SUB):
                v = rr[:, 128 * (t - t0):128 * (t - t0 + 1)] * scale[j][t]
                ctx[t] = v if ctx[t] is None else ctx[t] + v
        return jnp.concatenate([x.astype(BF) for x in ctx], axis=1)

    def router():
        rows = lax.broadcasted_iota(jnp.int32, (16, M), 0)
        wr = jnp.broadcast_to(wr_ref[...].reshape(1, M).astype(F32), (16, M))
        gw = jnp.broadcast_to(gw_ref[...].reshape(1, M).astype(F32), (16, M))
        lhs = jnp.where(rows == 0, wr, jnp.where(rows == 1, gw, 0.0)).astype(BF)
        xt = _up(xT[...])
        rz = _dot(lhs, xt, NN)
        g_s[...] = jax.nn.sigmoid(rz[1:2, :])
        rt = rz[0:1, :].astype(BF).astype(F32)
        tok = lax.broadcasted_iota(jnp.int32, (1, S), 1)
        m0 = jnp.max(rt, axis=1, keepdims=True)
        i0 = jnp.min(jnp.where(rt == m0, tok, S), axis=1, keepdims=True)
        rt1 = jnp.where(tok == i0, -jnp.inf, rt)
        m1 = jnp.max(rt1, axis=1, keepdims=True)
        i1 = jnp.min(jnp.where((rt1 == m1) & (tok != i0), tok, S), axis=1, keepdims=True)
        r16 = lax.broadcasted_iota(jnp.int32, (16, S), 0)
        t16 = lax.broadcasted_iota(jnp.int32, (16, S), 1)
        want = jnp.where(r16 == 0, i0, jnp.where(r16 == 1, i1, -1))
        onehot = jnp.where(t16 == want, 1.0, 0.0).astype(BF)
        xsel[...] = _pk(_dot(onehot, xt, NT).astype(BF))
        r8 = lax.broadcasted_iota(jnp.int32, (8, 128), 0)
        i0b = jnp.broadcast_to(i0.astype(F32), (8, 128))
        i1b = jnp.broadcast_to(i1.astype(F32), (8, 128))
        s0b = jnp.broadcast_to(jax.nn.sigmoid(m0), (8, 128))
        s1b = jnp.broadcast_to(jax.nn.sigmoid(m1), (8, 128))
        sel_s[...] = jnp.where(r8 == 0, i0b, jnp.where(r8 == 1, i1b, jnp.where(r8 == 2, s0b, s1b)))
        y_s[...] = jnp.zeros_like(y_s)

    def ffn_chunk(h):
        cols = pl.ds(pl.multiple_of(jnp.minimum(h, NF - 1) * FT, FT), FT)
        xs = _up(xsel[...])
        gg = _dot(xs, _up(wg[:, cols]), NN)
        uu = _dot(xs, _up(wu[:, cols]), NN)
        hh = (gg * jax.nn.sigmoid(gg) * uu).astype(BF)
        y_s[...] += jnp.where(h < NF, _dot(hh, _up(wdT[:, cols]), NT), 0.0)

    wq_copy(0, 0).start()
    for i in range(S // XW):
        x_copy(i).start()
    wk_copy(0, 0).start()
    wv_copy(0, 0).start()
    for i in range(NQ):
        c_copy(i).start()
    for cp in side_copies(True):
        cp.start()
    acc[...] = jnp.zeros_like(acc)

    wq_copy(0, 0).wait()
    for j in range(4):
        prep_q(0, 0, 128 * j, min(128, M - 128 * j))

    def q_first(i, carry):
        x_copy(i).wait()
        projq(pl.multiple_of(i * XW, XW), XW)
        return carry
    lax.fori_loop(0, S // XW, q_first, 0)
    router()

    wk_copy(0, 0).wait()
    wv_copy(0, 0).wait()

    def prep_first(j, carry):
        r0 = pl.multiple_of(j * 128, 128)
        wkb[pl.ds(pl.multiple_of(j * 64, 64), 64), :] = _pk(_head_of_pair(wk32[0, pl.ds(r0, 128), :], 0).astype(BF))
        prep_v(0, 0, r0, 128)
        return carry
    lax.fori_loop(0, DC // 128, prep_first, 0)

    wq_copy(1, 1).start()
    wk_copy(1, 1).start()
    wv_copy(1, 1).start()
    for cp in side_copies(False):
        cp.start()

    def kv_first(i, carry):
        c_copy(i).wait()
        rp = pl.ds(pl.multiple_of(i * (TQ // 2), TQ // 2), TQ // 2)
        cc = _up(c[rp, :])
        k_s[rp, :] = _pk(_dot(cc, _up(wkb[...]), NN).astype(BF))
        vT[:, pl.ds(pl.multiple_of(i * TQ, TQ), TQ)] = _pk(_dot(_up(wvT[...]), cc, NT).astype(BF))
        return carry
    lax.fori_loop(0, NQ, kv_first, 0)
    for cp in side_copies(True):
        cp.wait()

    def head_step(h, carry):
        pn = (h + 1) // 2

        @pl.when(h % 2 == 1)
        def _():
            sl = pn % 2
            wq_copy(pn, sl).wait()
            wk_copy(pn, sl).wait()
            wv_copy(pn, sl).wait()

            @pl.when(pn + 1 < H // 2)
            def _():
                wq_copy(pn + 1, 1 - sl).start()
                wk_copy(pn + 1, 1 - sl).start()
                wv_copy(pn + 1, 1 - sl).start()

        @pl.when(h == 1)
        def _():
            for cp in side_copies(False):
                cp.wait()

        prep_all(pn % 2, (h + 1) % 2)
        wo = _up(woT[h])
        pp = scores(NQ - 1)
        ffn_chunk(h)
        for i in range(NQ - 1, -1, -1):
            pnext = scores(i - 1) if i > 0 else None
            cb = context(pp)
            projk(i * TQ)
            acc[:, pl.ds(i * TQ, TQ)] += _dot(wo, cb, NN)
            projq(i * TQ)
            projv(i * TQ)
            pp = pnext
        return carry

    lax.fori_loop(0, H - 1, head_step, 0)

    sel = sel_s[...]
    yT = y_s[...].T
    y0 = yT[:, 0:1] * sel[2:3, 0:1]
    y1 = yT[:, 1:2] * sel[3:4, 0:1]
    wo = _up(woT[H - 1])

    def finish(i, cb):
        r = pl.ds(i * TQ, TQ)
        a = acc[:, r] + _dot(wo, cb, NN)
        tok = (lax.broadcasted_iota(jnp.int32, (1, TQ), 1) + i * TQ).astype(F32)
        b = _up(xT[:, r]).astype(F32)
        b = b + jnp.where(tok == sel[0:1, 0:1], y0, jnp.where(tok == sel[1:2, 0:1], y1, 0.0))
        g = g_s[:, r]
        obuf[:, r] = _pk((g * a + (1.0 - g) * b).astype(BF))

    pp = scores(NQ - 1)
    pnext = scores(NQ - 2)
    for i in range(NQ - 1, -1, -1):
        cb = context(pp)
        pp = pnext
        pnext = scores(i - 2) if i >= 2 else None
        finish(i, cb)
    for i in range(NQ - 1, -1, -1):
        o_copy(i).start()
    for i in range(NQ - 1, -1, -1):
        o_copy(i).wait()


@jax.jit
def pallas_gated_mix__compressed_kv_cla__moe_arch_mod__prompt_kernel(
        A_x, A_c_kv, A_w_q, A_w_uk, A_w_uv, A_w_o, B_x, B_w_r, B_w_gate, B_w_up, B_w_down, gate_w):
    xT = jnp.transpose(A_x, (0, 2, 1)).reshape(M, S)
    c = A_c_kv.reshape(S, DC)
    woT = jnp.transpose(A_w_o, (0, 2, 1))
    wdT = B_w_down.T
    hbm = pl.BlockSpec(memory_space=pltpu.HBM)
    vec = pl.BlockSpec(memory_space=pltpu.VMEM)
    outT = pl.pallas_call(
        _kernel,
        in_specs=[hbm, hbm, hbm, hbm, hbm, hbm, vec, vec, hbm, hbm, hbm],
        out_specs=hbm,
        out_shape=jax.ShapeDtypeStruct((M, S), BF),
        scratch_shapes=[
            pltpu.VMEM((M // 2, S), U32),
            pltpu.VMEM((S // 2, DC), U32),
            pltpu.VMEM((2, M, D), U32),
            pltpu.VMEM((2, DC, D), U32),
            pltpu.VMEM((2, DC, D), U32),
            pltpu.VMEM((H, M // 2, D), U32),
            pltpu.VMEM((M // 2, F), U32),
            pltpu.VMEM((M // 2, F), U32),
            pltpu.VMEM((M // 2, F), U32),
            pltpu.VMEM((D // 2, M), U32),
            pltpu.VMEM((DC // 2, D), U32),
            pltpu.VMEM((D // 2, DC), U32),
            pltpu.VMEM((D // 2, S), U32),
            pltpu.VMEM((S // 2, D), U32),
            pltpu.VMEM((D // 2, S), U32),
            pltpu.VMEM((M, S), F32),
            pltpu.VMEM((M // 2, S), U32),
            pltpu.VMEM((8, M), U32),
            pltpu.VMEM((16, M), F32),
            pltpu.VMEM((8, 128), F32),
            pltpu.VMEM((1, S), F32),
            pltpu.SemaphoreType.DMA((2, 3)),
            pltpu.SemaphoreType.DMA((NQ,)),
            pltpu.SemaphoreType.DMA((4,)),
            pltpu.SemaphoreType.DMA((8,)),
            pltpu.SemaphoreType.DMA((NQ,)),
        ],
        compiler_params=pltpu.CompilerParams(vmem_limit_bytes=100 * 1024 * 1024),
        name="gated_mix",
    )(xT, c, A_w_q, A_w_uk, A_w_uv, woT, B_w_r, gate_w, B_w_gate, B_w_up, wdT)
    return jnp.transpose(outT.reshape(1, M, S), (0, 2, 1))
```

```python
import functools
import jax
import jax.numpy as jnp
from jax import lax
from jax.experimental import pallas as pl
from jax.experimental.pallas import tpu as pltpu

S = 2048
M = 448
DC = 1024
H = 16
D = 256
F = 1792
FT = 128
NF = F // FT
TQ = 256
NQ = S // TQ
SUB = TQ // 128
FFN_UP, FFN_DOWN = 5, 3
OMID = 5
O3 = 1
LOG2E = 1.4426950408889634
QSCALE = (D ** -0.5) * LOG2E
NEG = -1e9 * LOG2E
BF = jnp.bfloat16
F32 = jnp.float32
U32 = jnp.uint32

NT = (((1,), (1,)), ((), ()))
NN = (((1,), (0,)), ((), ()))
_dot = functools.partial(lax.dot_general, preferred_element_type=F32)


def _pk(x):
    return pltpu.bitcast(x, U32)


def _up(x):
    return pltpu.bitcast(x, BF)


def _rows(start, n):
    return pl.ds(start // 2, n // 2)


def _head_of_pair(w32, parity):
    if isinstance(parity, int):
        bits = (w32 << 16) if parity == 0 else (w32 & jnp.uint32(0xFFFF0000))
    else:
        sh = (16 - 16 * parity).astype(U32)
        bits = lax.shift_left(w32, jnp.broadcast_to(sh, w32.shape)) & jnp.uint32(0xFFFF0000)
    return pltpu.bitcast(bits, F32)


def _kernel(xT_hbm, c_hbm, wq_hbm, wk_hbm, wv_hbm, woT_hbm, wr_hbm, gw_hbm,
            wg_hbm, wu_hbm, wdT_hbm, oT_hbm,
            xT, c, wq32, wk32, wv32, woT, wg, wu, wdT, wqT, wkb, wvT, qT, k_s, vT, acc, obuf,
            xsel, y_s, sel_s, g_s, rrows, rz_s, wr_ref, gw_ref, idx_s, wsem, csem, xsem, msem, osem):

    def wq_copy(p, sl):
        return pltpu.make_async_copy(wq_hbm.bitcast(U32).at[:, p, :], wq32.at[sl], wsem.at[sl, 0])

    def wk_copy(p, sl):
        return pltpu.make_async_copy(wk_hbm.bitcast(U32).at[:, p, :], wk32.at[sl], wsem.at[sl, 1])

    def wv_copy(p, sl):
        return pltpu.make_async_copy(wv_hbm.bitcast(U32).at[:, p, :], wv32.at[sl], wsem.at[sl, 2])

    def c_copy(i):
        r = pl.ds(i * (TQ // 2), TQ // 2)
        return pltpu.make_async_copy(c_hbm.bitcast(U32).at[r, :], c.at[r, :], csem.at[i])

    XW = 512
    def x_copy(i):
        r = pl.ds(i * XW, XW)
        return pltpu.make_async_copy(xT_hbm.bitcast(U32).at[:, r], xT.at[:, r], xsem.at[i])

    def side_copies(first):
        hs = pl.ds(0, 1) if first else pl.ds(1, H - 1)
        cs = pl.ds(0, FT) if first else pl.ds(FT, F - FT)
        o = 0 if first else 4
        return [pltpu.make_async_copy(woT_hbm.bitcast(U32).at[hs], woT.at[hs], msem.at[o]),
                pltpu.make_async_copy(wg_hbm.bitcast(U32).at[:, cs], wg.at[:, cs], msem.at[o + 1]),
                pltpu.make_async_copy(wu_hbm.bitcast(U32).at[:, cs], wu.at[:, cs], msem.at[o + 2]),
                pltpu.make_async_copy(wdT_hbm.bitcast(U32).at[:, cs], wdT.at[:, cs], msem.at[o + 3])]

    def vec_copies():
        return [pltpu.make_async_copy(wr_hbm, wr_ref, msem.at[8]),
                pltpu.make_async_copy(gw_hbm, gw_ref, msem.at[9])]

    def o_copy(i, n, k):
        r = pl.ds(i * TQ, n * TQ)
        return pltpu.make_async_copy(obuf.at[:, r], oT_hbm.at[:, r], osem.at[k])

    def prep_k(sl, parity, r0, n):
        wkb[_rows(r0, n), :] = _pk(_head_of_pair(wk32[sl, pl.ds(r0, n), :], parity).astype(BF))

    def prep_v(sl, parity, r0, n):
        wvT[:, pl.ds(r0, n)] = _pk(_head_of_pair(wv32[sl, pl.ds(r0, n), :], parity).T.astype(BF))

    def prep_q(sl, parity, r0, n):
        wqT[:, pl.ds(r0, n)] = _pk(_head_of_pair(wq32[sl, pl.ds(r0, n), :], parity).T.astype(BF))

    def prep_all(sl, parity):
        for j in range(DC // 128):
            prep_k(sl, parity, 128 * j, 128)
        for j in range(4):
            prep_q(sl, parity, 128 * j, min(128, M - 128 * j))
        for j in range(DC // 128):
            prep_v(sl, parity, 128 * j, 128)

    def projk(r0):
        k_s[_rows(r0, TQ), :] = _pk(_dot(_up(c[_rows(r0, TQ), :]), _up(wkb[...]), NN).astype(BF))

    def projq(r0, n=TQ):
        r = pl.ds(r0, n)
        qT[:, r] = _pk((_dot(_up(wqT[...]), _up(xT[:, r]), NN) * QSCALE).astype(BF))

    def projv(r0):
        vT[:, pl.ds(r0, TQ)] = _pk(_dot(_up(wvT[...]), _up(c[_rows(r0, TQ), :]), NT).astype(BF))

    def split_dot(lhs_ref_rows, n, parts, rhs):
        w = n // parts
        rr = [_dot(lhs_ref_rows(w * u, w), rhs, NN) for u in range(parts)]
        return jnp.concatenate(rr, axis=0) if parts > 1 else rr[0]

    def scores(i, lone=False, mid=None):
        tri = (lax.broadcasted_iota(jnp.int32, (128, 128), 0)
               <= lax.broadcasted_iota(jnp.int32, (128, 128), 1))
        base = i * TQ
        q = _up(qT[:, pl.ds(base, TQ)])
        out = []
        for j in range(base // 128 + SUB):
            k0 = 128 * j
            if mid is not None and j == 2:
                mid()
            t0 = max(0, j - base // 128)
            s = split_dot(lambda a, n: _up(k_s[_rows(k0 + a, n), :]), 128,
                          2 if (lone and t0 == SUB - 1) else 1, q[:, 128 * t0:])
            if k0 >= base:
                blk = jnp.where(tri, s[:, 0:128], NEG)
                s = jnp.concatenate([blk, s[:, 128:]], axis=1) if SUB - t0 > 1 else blk
            m = jnp.max(s, axis=0, keepdims=True)
            e = jnp.exp2(s - m)
            out.append((t0, m, jnp.sum(e, axis=0, keepdims=True), e.astype(BF)))
        return out

    def context(i, chunks, lone=False, mid=None):
        scale = [[None] * SUB for _ in chunks]
        for t in range(SUB):
            js = [j for j, ch in enumerate(chunks) if ch[0] <= t]
            col = lambda x, j: x[:, 128 * (t - chunks[j][0]):128 * (t - chunks[j][0] + 1)]
            ms = [col(chunks[j][1], j) for j in js]
            m = functools.reduce(jnp.maximum, ms)
            al = [jnp.exp2(mj - m) for mj in ms]
            l = functools.reduce(jnp.add, [a * col(chunks[j][2], j) for a, j in zip(al, js)])
            li = g_s[:, pl.ds(i * TQ + 128 * t, 128)] / l
            for a, j in zip(al, js):
                scale[j][t] = a * li
        ctx = [None] * SUB
        n = len(chunks)
        for cnt, j in enumerate([n - 1, n - 2] + list(range(n - 2))):
            t0, _, _, p = chunks[j]
            parts = (4 if lone else 2) if j == n - 1 else (2 if j == n - 2 else 1)
            if mid is not None and cnt == 6:
                mid()
            rr = split_dot(lambda a, w: _up(vT[_rows(a, w), pl.ds(128 * j, 128)]), D, parts, p)
            for t in range(t0, SUB):
                v = rr[:, 128 * (t - t0):128 * (t - t0 + 1)] * scale[j][t]
                ctx[t] = v if ctx[t] is None else ctx[t] + v
        return jnp.concatenate(ctx, axis=1).astype(BF)

    def router_rows():
        rows = lax.broadcasted_iota(jnp.int32, (16, M), 0)
        wr = jnp.broadcast_to(wr_ref[...].reshape(1, M).astype(F32), (16, M))
        gw = jnp.broadcast_to(gw_ref[...].reshape(1, M).astype(F32), (16, M))
        return jnp.where(rows == 0, wr, jnp.where(rows == 1, gw, 0.0)).astype(BF)

    def router():
        rz = rz_s[...]
        g = jax.nn.sigmoid(rz[1:2, :])
        g_s[...] = g
        rt = rz[0:1, :].astype(BF).astype(F32)
        tok = lax.broadcasted_iota(jnp.int32, (1, S), 1)
        m0 = jnp.max(rt, axis=1, keepdims=True)
        i0 = jnp.min(jnp.where(rt == m0, tok, S - 1), axis=1, keepdims=True)
        rt1 = jnp.where(tok == i0, -jnp.inf, rt)
        m1 = jnp.max(rt1, axis=1, keepdims=True)
        i1 = jnp.min(jnp.where((rt1 == m1) & (tok != i0), tok, S - 1), axis=1, keepdims=True)
        r16 = lax.broadcasted_iota(jnp.int32, (16, 128), 0)
        l16 = lax.broadcasted_iota(jnp.int32, (16, 128), 1)
        xs = None
        wsel = []
        for row, idx, mx in ((0, i0, m0), (1, i1, m1)):
            si = jnp.max(idx)
            idx_s[row] = si
            tile = _up(xT[:, pl.ds(pl.multiple_of((si >> 7) * 128, 128), 128)])
            onehot = jnp.where((r16 == row) & (l16 == (idx & 127)), 1.0, 0.0).astype(BF)
            part = _dot(onehot, tile, NT)
            xs = part if xs is None else xs + part
            keep = jnp.sum(jnp.where(tok == idx, 1.0 - g, 0.0), axis=1, keepdims=True)
            wsel.append(jnp.broadcast_to(jax.nn.sigmoid(mx) * keep, (8, 128)))
        xsel[...] = _pk(xs.astype(BF))
        r8 = lax.broadcasted_iota(jnp.int32, (8, 128), 0)
        sel_s[...] = jnp.where(r8 == 0, wsel[0], wsel[1])
        y_s[...] = jnp.zeros_like(y_s)

    def ffn_up(h):
        cols = pl.ds(pl.multiple_of(jnp.minimum(h, NF - 1) * FT, FT), FT)
        xs = _up(xsel[...])
        gg = _dot(xs, _up(wg[:, cols]), NN)
        uu = _dot(xs, _up(wu[:, cols]), NN)
        return (gg * jax.nn.sigmoid(gg) * uu).astype(BF)

    def ffn_down(h, hh):
        cols = pl.ds(pl.multiple_of(jnp.minimum(h, NF - 1) * FT, FT), FT)
        y_s[...] += jnp.where(h < NF, _dot(hh, _up(wdT[:, cols]), NT), 0.0)

    wq_copy(0, 0).start()
    for cp in vec_copies():
        cp.start()
    for i in range(S // XW):
        x_copy(i).start()
    wk_copy(0, 0).start()
    for i in range(NQ):
        c_copy(i).start()
    wv_copy(0, 0).start()
    for cp in side_copies(True):
        cp.start()
    wq_copy(1, 1).start()
    wk_copy(1, 1).start()
    wv_copy(1, 1).start()
    for cp in side_copies(False):
        cp.start()
    acc[...] = jnp.zeros_like(acc)

    wq_copy(0, 0).wait()
    for cp in vec_copies():
        cp.wait()
    rrows[...] = _pk(router_rows())
    for j in range(4):
        prep_q(0, 0, 128 * j, min(128, M - 128 * j))

    def q_first(i, carry):
        x_copy(i).wait()
        r = pl.ds(pl.multiple_of(i * XW, XW), XW)
        lhs = jnp.concatenate([_up(wqT[...]), _up(rrows[...])], axis=0)
        res = _dot(lhs, _up(xT[:, r]), NN)
        qT[:, r] = _pk((res[:D] * QSCALE).astype(BF))
        rz_s[:, r] = res[D:D + 8]
        return carry
    lax.fori_loop(0, S // XW, q_first, 0)
    router()

    wk_copy(0, 0).wait()
    for j in range(DC // 128):
        prep_k(0, 0, 128 * j, 128)

    def k_first(i, carry):
        c_copy(i).wait()
        rp = pl.ds(pl.multiple_of(i * (TQ // 2), TQ // 2), TQ // 2)
        k_s[rp, :] = _pk(_dot(_up(c[rp, :]), _up(wkb[...]), NN).astype(BF))
        return carry
    lax.fori_loop(0, NQ, k_first, 0)

    wv_copy(0, 0).wait()
    for j in range(DC // 128):
        prep_v(0, 0, 128 * j, 128)

    VW = 512
    def v_first(i, carry):
        rp = pl.ds(pl.multiple_of(i * (VW // 2), VW // 2), VW // 2)
        vT[:, pl.ds(pl.multiple_of(i * VW, VW), VW)] = _pk(_dot(_up(wvT[...]), _up(c[rp, :]), NT).astype(BF))
        return carry
    lax.fori_loop(0, S // VW, v_first, 0)
    for cp in side_copies(True):
        cp.wait()

    def head_step(h, carry):
        pn = (h + 1) >> 1

        @pl.when((h & 1) == 1)
        def _():
            wq_copy(pn, pn & 1).wait()
            wk_copy(pn, pn & 1).wait()
            wv_copy(pn, pn & 1).wait()

        @pl.when(h == 1)
        def _():
            for cp in side_copies(False):
                cp.wait()

        prep_all(pn & 1, (h + 1) & 1)
        wo = _up(woT[h])
        pp = scores(NQ - 1, lone=True)
        for i in range(NQ - 1, -1, -1):
            pnext = scores(i - 1) if i > 0 else None
            cb = context(i, pp, lone=(i == 0))
            projk(i * TQ)
            acc[:, pl.ds(i * TQ, TQ)] += _dot(wo, cb, NN)
            if i == FFN_UP:
                hh = ffn_up(h)
            projq(i * TQ)
            if i == FFN_DOWN:
                ffn_down(h, hh)
            projv(i * TQ)
            pp = pnext

        @pl.when(jnp.logical_and((h & 1) == 0, pn + 2 < H // 2))
        def _():
            wq_copy(pn + 2, pn & 1).start()
            wk_copy(pn + 2, pn & 1).start()
            wv_copy(pn + 2, pn & 1).start()
        return carry

    lax.fori_loop(0, H - 1, head_step, 0)

    sel = sel_s[...]
    yT = y_s[...].T
    lane = lax.broadcasted_iota(jnp.int32, (1, 128), 1)
    for row in range(2):
        si = idx_s[row]
        r = pl.ds(pl.multiple_of((si >> 7) * 128, 128), 128)
        upd = yT[:, row:row + 1] * sel[row:row + 1, 0:1]
        acc[:, r] += jnp.where(lane == (si & 127), upd, 0.0)
    wo = _up(woT[H - 1])

    def finish(i, cb):
        r = pl.ds(i * TQ, TQ)
        res = (1.0 - g_s[:, r]) * _up(xT[:, r]).astype(F32)
        obuf[:, r] = (acc[:, r] + res + _dot(wo, cb, NN)).astype(BF)
        if i == OMID:
            o_copy(0, OMID + 1, 0).start()

    pp = scores(0, lone=True)
    pnext = scores(1)
    cb = context(0, pp)
    for i in range(1, NQ - 1):
        pp = pnext
        pnext = scores(i + 1, mid=functools.partial(finish, i - 1, cb))
        cb = context(i, pp)
    cb2 = context(NQ - 1, pnext, lone=True)
    finish(NQ - 2, cb)
    if O3:
        o_copy(OMID + 1, NQ - OMID - 2, 2).start()
    finish(NQ - 1, cb2)
    if O3:
        o_copy(NQ - 1, 1, 1).start()
        o_copy(OMID + 1, NQ - OMID - 2, 2).wait()
        o_copy(NQ - 1, 1, 1).wait()
    else:
        o_copy(OMID + 1, NQ - OMID - 1, 1).start()
        o_copy(OMID + 1, NQ - OMID - 1, 1).wait()
    o_copy(0, OMID + 1, 0).wait()


@jax.jit
def pallas_gated_mix__compressed_kv_cla__moe_arch_mod__prompt_kernel(
        A_x, A_c_kv, A_w_q, A_w_uk, A_w_uv, A_w_o, B_x, B_w_r, B_w_gate, B_w_up, B_w_down, gate_w):
    xT = jnp.transpose(A_x, (0, 2, 1)).reshape(M, S)
    c = A_c_kv.reshape(S, DC)
    woT = jnp.transpose(A_w_o, (0, 2, 1))
    wdT = B_w_down.T
    hbm = pl.BlockSpec(memory_space=pltpu.HBM)
    outT = pl.pallas_call(
        _kernel,
        in_specs=[hbm] * 11,
        out_specs=hbm,
        out_shape=jax.ShapeDtypeStruct((M, S), BF),
        scratch_shapes=[
            pltpu.VMEM((M // 2, S), U32),
            pltpu.VMEM((S // 2, DC), U32),
            pltpu.VMEM((2, M, D), U32),
            pltpu.VMEM((2, DC, D), U32),
            pltpu.VMEM((2, DC, D), U32),
            pltpu.VMEM((H, M // 2, D), U32),
            pltpu.VMEM((M // 2, F), U32),
            pltpu.VMEM((M // 2, F), U32),
            pltpu.VMEM((M // 2, F), U32),
            pltpu.VMEM((D // 2, M), U32),
            pltpu.VMEM((DC // 2, D), U32),
            pltpu.VMEM((D // 2, DC), U32),
            pltpu.VMEM((D // 2, S), U32),
            pltpu.VMEM((S // 2, D), U32),
            pltpu.VMEM((D // 2, S), U32),
            pltpu.VMEM((M, S), F32),
            pltpu.VMEM((M, S), BF),
            pltpu.VMEM((8, M), U32),
            pltpu.VMEM((16, M), F32),
            pltpu.VMEM((8, 128), F32),
            pltpu.VMEM((1, S), F32),
            pltpu.VMEM((8, M), U32),
            pltpu.VMEM((8, S), F32),
            pltpu.VMEM((M,), BF),
            pltpu.VMEM((M,), BF),
            pltpu.SMEM((2,), jnp.int32),
            pltpu.SemaphoreType.DMA((2, 3)),
            pltpu.SemaphoreType.DMA((NQ,)),
            pltpu.SemaphoreType.DMA((4,)),
            pltpu.SemaphoreType.DMA((10,)),
            pltpu.SemaphoreType.DMA((3,)),
        ],
        compiler_params=pltpu.CompilerParams(vmem_limit_bytes=100 * 1024 * 1024,
                                             disable_bounds_checks=True,
                                             disable_semaphore_checks=True),
        name="gated_mix",
    )(xT, c, A_w_q, A_w_uk, A_w_uv, woT, B_w_r, gate_w, B_w_gate, B_w_up, wdT)
    return jnp.transpose(outT.reshape(1, M, S), (0, 2, 1))
```

```python
import functools
import jax
import jax.numpy as jnp
from jax import lax
from jax.experimental import pallas as pl
from jax.experimental.pallas import tpu as pltpu

S = 2048
M = 448
DC = 1024
H = 16
D = 256
F = 1792
FT = 128
NF = F // FT
TQ = 256
NQ = S // TQ
SUB = TQ // 128
FFN_UP, FFN_DOWN = 5, 3
QKG = 2
OMID = 5
NK0 = 2
O3 = 1
LOG2E = 1.4426950408889634
QSCALE = (D ** -0.5) * LOG2E
NEG = -1e9 * LOG2E
BF = jnp.bfloat16
F32 = jnp.float32
U32 = jnp.uint32

NT = (((1,), (1,)), ((), ()))
NN = (((1,), (0,)), ((), ()))
_dot = functools.partial(lax.dot_general, preferred_element_type=F32)


def _pk(x):
    return pltpu.bitcast(x, U32)


def _up(x):
    return pltpu.bitcast(x, BF)


def _rows(start, n):
    return pl.ds(start // 2, n // 2)


def _token_tile(tok):
    t = jnp.clip(tok >> 7, 0, S // 128 - 1)
    return pl.ds(pl.multiple_of(t * 128, 128), 128)


def _head_of_pair(w32, parity):
    if isinstance(parity, int):
        bits = (w32 << 16) if parity == 0 else (w32 & jnp.uint32(0xFFFF0000))
    else:
        sh = (16 - 16 * parity).astype(U32)
        bits = lax.shift_left(w32, jnp.broadcast_to(sh, w32.shape)) & jnp.uint32(0xFFFF0000)
    return pltpu.bitcast(bits, F32)


def _kernel(xT_hbm, c_hbm, wq_hbm, wk_hbm, wv_hbm, woT_hbm, wr_hbm, gw_hbm,
            wg_hbm, wu_hbm, wdT_hbm, oT_hbm,
            xT, c, wq32, wk32, wv32, woT, wg, wu, wdT, wqT, wkb, wvT, qT, k_s, vT, acc, obuf,
            xsel, y_s, sel_s, g_s, rrows, rz_s, wr_ref, gw_ref, idx_s, wo_s, wsem, csem, xsem, msem, osem):

    def wq_copy(p, sl):
        return pltpu.make_async_copy(wq_hbm.bitcast(U32).at[:, p, :], wq32.at[sl], wsem.at[sl, 0])

    def wk_copy(p, sl):
        return pltpu.make_async_copy(wk_hbm.bitcast(U32).at[:, p, :], wk32.at[sl], wsem.at[sl, 1])

    def wv_copy(p, sl):
        return pltpu.make_async_copy(wv_hbm.bitcast(U32).at[:, p, :], wv32.at[sl], wsem.at[sl, 2])

    def c_copy(i):
        r = pl.ds(i * (TQ // 2), TQ // 2)
        return pltpu.make_async_copy(c_hbm.bitcast(U32).at[r, :], c.at[r, :], csem.at[i])

    XW = 512
    def x_copy(i):
        r = pl.ds(i * XW, XW)
        return pltpu.make_async_copy(xT_hbm.bitcast(U32).at[:, r], xT.at[:, r], xsem.at[i])

    def side_copies(first):
        hs = pl.ds(0, 1) if first else pl.ds(1, H - 1)
        cs = pl.ds(0, FT) if first else pl.ds(FT, F - FT)
        o = 0 if first else 4
        return [pltpu.make_async_copy(woT_hbm.bitcast(U32).at[hs], woT.at[hs], msem.at[o]),
                pltpu.make_async_copy(wg_hbm.bitcast(U32).at[:, cs], wg.at[:, cs], msem.at[o + 1]),
                pltpu.make_async_copy(wu_hbm.bitcast(U32).at[:, cs], wu.at[:, cs], msem.at[o + 2]),
                pltpu.make_async_copy(wdT_hbm.bitcast(U32).at[:, cs], wdT.at[:, cs], msem.at[o + 3])]

    def vec_copies():
        return [pltpu.make_async_copy(wr_hbm, wr_ref, msem.at[8]),
                pltpu.make_async_copy(gw_hbm, gw_ref, msem.at[9])]

    def o_copy(i, n, k):
        r = pl.ds(i * TQ, n * TQ)
        return pltpu.make_async_copy(obuf.at[:, r], oT_hbm.at[:, r], osem.at[k])

    def prep_k(sl, parity, r0, n):
        wkb[_rows(r0, n), :] = _pk(_head_of_pair(wk32[sl, pl.ds(r0, n), :], parity).astype(BF))

    def prep_v(sl, parity, r0, n):
        wvT[:, pl.ds(r0, n)] = _pk(_head_of_pair(wv32[sl, pl.ds(r0, n), :], parity).T.astype(BF))

    def prep_q(sl, parity, r0, n):
        wqT[:, pl.ds(r0, n)] = _pk(_head_of_pair(wq32[sl, pl.ds(r0, n), :], parity).T.astype(BF))

    def prep_all(sl, parity):
        for j in range(DC // 128):
            prep_k(sl, parity, 128 * j, 128)
        for j in range(4):
            prep_q(sl, parity, 128 * j, min(128, M - 128 * j))
        for j in range(DC // 128):
            prep_v(sl, parity, 128 * j, 128)

    def projk(r0):
        k_s[_rows(r0, TQ), :] = _pk(_dot(_up(c[_rows(r0, TQ), :]), _up(wkb[...]), NN).astype(BF))

    def projq(r0, n=TQ):
        r = pl.ds(r0, n)
        qT[:, r] = _pk((_dot(_up(wqT[...]), _up(xT[:, r]), NN) * QSCALE).astype(BF))

    def projv(r0):
        vT[:, pl.ds(r0, TQ)] = _pk(_dot(_up(wvT[...]), _up(c[_rows(r0, TQ), :]), NT).astype(BF))

    def split_dot(lhs_ref_rows, n, parts, rhs):
        w = n // parts
        rr = [_dot(lhs_ref_rows(w * u, w), rhs, NN) for u in range(parts)]
        return jnp.concatenate(rr, axis=0) if parts > 1 else rr[0]

    def scores(i, lone=False, mid=None):
        tri = (lax.broadcasted_iota(jnp.int32, (128, 128), 0)
               <= lax.broadcasted_iota(jnp.int32, (128, 128), 1))
        base = i * TQ
        out = []
        nfull = base // 128
        big = {}
        for j in range(nfull + SUB):
            k0 = 128 * j
            if mid is not None and j == 2:
                mid()
            t0 = max(0, j - nfull)
            if j < nfull and QKG > 1:
                if j % QKG == 0:
                    n = min(QKG, nfull - j)
                    sb = _dot(_up(k_s[_rows(k0, 128 * n), :]), _up(qT[:, pl.ds(base, TQ)]), NN)
                s = sb[128 * (j % QKG):128 * (j % QKG + 1)]
            else:
                s = split_dot(lambda a, n: _up(k_s[_rows(k0 + a, n), :]), 128,
                              2 if (lone and t0 == SUB - 1) else 1,
                              _up(qT[:, pl.ds(base + 128 * t0, TQ - 128 * t0)]))
            if k0 >= base:
                blk = jnp.where(tri, s[:, 0:128], NEG)
                s = jnp.concatenate([blk, s[:, 128:]], axis=1) if SUB - t0 > 1 else blk
            m = jnp.max(s, axis=0, keepdims=True)
            e = jnp.exp2(s - m)
            out.append((t0, m, jnp.sum(e, axis=0, keepdims=True), e.astype(BF)))
        return out

    def context(i, chunks, lone=False, mid=None):
        scale = [[None] * SUB for _ in chunks]
        for t in range(SUB):
            js = [j for j, ch in enumerate(chunks) if ch[0] <= t]
            col = lambda x, j: x[:, 128 * (t - chunks[j][0]):128 * (t - chunks[j][0] + 1)]
            ms = [col(chunks[j][1], j) for j in js]
            m = functools.reduce(jnp.maximum, ms)
            al = [jnp.exp2(mj - m) for mj in ms]
            l = functools.reduce(jnp.add, [a * col(chunks[j][2], j) for a, j in zip(al, js)])
            li = g_s[:, pl.ds(i * TQ + 128 * t, 128)] / l
            for a, j in zip(al, js):
                scale[j][t] = a * li
        ctx = [None] * SUB
        n = len(chunks)
        for cnt, j in enumerate([n - 1, n - 2] + list(range(n - 2))):
            t0, _, _, p = chunks[j]
            parts = (4 if lone else 2) if j == n - 1 else (2 if j == n - 2 else 1)
            if mid is not None and cnt == 6:
                mid()
            rr = split_dot(lambda a, w: _up(vT[_rows(a, w), pl.ds(128 * j, 128)]), D, parts, p)
            for t in range(t0, SUB):
                v = rr[:, 128 * (t - t0):128 * (t - t0 + 1)] * scale[j][t]
                ctx[t] = v if ctx[t] is None else ctx[t] + v
        return jnp.concatenate(ctx, axis=1).astype(BF)

    def router_rows():
        rows = lax.broadcasted_iota(jnp.int32, (16, M), 0)
        wr = jnp.broadcast_to(wr_ref[...].reshape(1, M).astype(F32), (16, M))
        gw = jnp.broadcast_to(gw_ref[...].reshape(1, M).astype(F32), (16, M))
        return jnp.where(rows == 0, wr, jnp.where(rows == 1, gw, 0.0)).astype(BF)

    def router():
        rz = rz_s[...]
        g = jax.nn.sigmoid(rz[1:2, :])
        g_s[...] = g
        rt = rz[0:1, :].astype(BF).astype(F32)
        tok = lax.broadcasted_iota(jnp.int32, (1, S), 1)
        m0 = jnp.max(rt, axis=1, keepdims=True)
        i0 = jnp.min(jnp.where(rt == m0, tok, S - 1), axis=1, keepdims=True)
        rt1 = jnp.where(tok == i0, -jnp.inf, rt)
        m1 = jnp.max(rt1, axis=1, keepdims=True)
        i1 = jnp.min(jnp.where((rt1 == m1) & (tok != i0), tok, S - 1), axis=1, keepdims=True)
        r16 = lax.broadcasted_iota(jnp.int32, (16, 128), 0)
        l16 = lax.broadcasted_iota(jnp.int32, (16, 128), 1)
        xs = None
        wsel = []
        for row, idx, mx in ((0, i0, m0), (1, i1, m1)):
            si = jnp.max(idx)
            idx_s[row] = si
            tile = _up(xT[:, _token_tile(si)])
            onehot = jnp.where((r16 == row) & (l16 == (idx & 127)), 1.0, 0.0).astype(BF)
            part = _dot(onehot, tile, NT)
            xs = part if xs is None else xs + part
            keep = jnp.sum(jnp.where(tok == idx, 1.0 - g, 0.0), axis=1, keepdims=True)
            wsel.append(jnp.broadcast_to(jax.nn.sigmoid(mx) * keep, (8, 128)))
        xsel[...] = _pk(xs.astype(BF))
        r8 = lax.broadcasted_iota(jnp.int32, (8, 128), 0)
        sel_s[...] = jnp.where(r8 == 0, wsel[0], wsel[1])
        y_s[...] = jnp.zeros_like(y_s)

    def ffn_up(h):
        cols = pl.ds(pl.multiple_of(jnp.minimum(h, NF - 1) * FT, FT), FT)
        xs = _up(xsel[...])
        gg = _dot(xs, _up(wg[:, cols]), NN)
        uu = _dot(xs, _up(wu[:, cols]), NN)
        return (gg * jax.nn.sigmoid(gg) * uu).astype(BF)

    def ffn_down(h, hh):
        cols = pl.ds(pl.multiple_of(jnp.minimum(h, NF - 1) * FT, FT), FT)
        y_s[...] += jnp.where(h < NF, _dot(hh, _up(wdT[:, cols]), NT), 0.0)

    wq_copy(0, 0).start()
    for cp in vec_copies():
        cp.start()
    for i in range(S // XW):
        x_copy(i).start()
    wk_copy(0, 0).start()
    for i in range(NQ):
        c_copy(i).start()
        if i == NK0 - 1:
            wv_copy(0, 0).start()
    for cp in side_copies(True):
        cp.start()
    wq_copy(1, 1).start()
    wk_copy(1, 1).start()
    wv_copy(1, 1).start()
    for cp in side_copies(False):
        cp.start()
    acc[...] = jnp.zeros_like(acc)

    wq_copy(0, 0).wait()
    for cp in vec_copies():
        cp.wait()
    rrows[...] = _pk(router_rows())
    for j in range(4):
        prep_q(0, 0, 128 * j, min(128, M - 128 * j))

    def q_first(i, carry):
        x_copy(i).wait()
        r = pl.ds(pl.multiple_of(i * XW, XW), XW)
        lhs = jnp.concatenate([_up(wqT[...]), _up(rrows[...])], axis=0)
        res = _dot(lhs, _up(xT[:, r]), NN)
        qT[:, r] = _pk((res[:D] * QSCALE).astype(BF))
        rz_s[:, r] = res[D:D + 8]
        return carry
    lax.fori_loop(0, S // XW, q_first, 0)

    wk_copy(0, 0).wait()
    for j in range(DC // 128):
        prep_k(0, 0, 128 * j, 128)

    def k_first(i, carry):
        c_copy(i).wait()
        rp = pl.ds(pl.multiple_of(i * (TQ // 2), TQ // 2), TQ // 2)
        k_s[rp, :] = _pk(_dot(_up(c[rp, :]), _up(wkb[...]), NN).astype(BF))
        return carry
    lax.fori_loop(0, NK0, k_first, 0)

    wv_copy(0, 0).wait()
    for j in range(DC // 128):
        prep_v(0, 0, 128 * j, 128)

    VW = 512
    vT[:, pl.ds(0, VW)] = _pk(_dot(_up(wvT[...]), _up(c[_rows(0, VW), :]), NT).astype(BF))
    router()

    def kv_first(i, carry):
        c_copy(2 * i).wait()
        c_copy(2 * i + 1).wait()
        rp = pl.ds(pl.multiple_of(i * (VW // 2), VW // 2), VW // 2)
        k_s[rp, :] = _pk(_dot(_up(c[rp, :]), _up(wkb[...]), NN).astype(BF))
        vT[:, pl.ds(pl.multiple_of(i * VW, VW), VW)] = _pk(_dot(_up(wvT[...]), _up(c[rp, :]), NT).astype(BF))
        return carry
    lax.fori_loop(1, S // VW, kv_first, 0)
    for cp in side_copies(True):
        cp.wait()

    def head_step(h, carry):
        pn = (h + 1) >> 1

        @pl.when((h & 1) == 1)
        def _():
            wq_copy(pn, pn & 1).wait()
            wk_copy(pn, pn & 1).wait()
            wv_copy(pn, pn & 1).wait()

            @pl.when(pn + 1 < H // 2)
            def _():
                wq_copy(pn + 1, 1 - (pn & 1)).start()
                wk_copy(pn + 1, 1 - (pn & 1)).start()
                wv_copy(pn + 1, 1 - (pn & 1)).start()

            @pl.when(h == 1)
            def _():
                for cp in side_copies(False):
                    cp.wait()

        prep_all(pn & 1, (h + 1) & 1)
        wo_s[...] = woT[h]
        pp = scores(NQ - 1, lone=True)
        projq((NQ - 1) * TQ)
        for i in range(NQ - 1, -1, -1):
            pnext = scores(i - 1) if i > 0 else None
            cb = context(i, pp, lone=(i == 0))
            projk(i * TQ)
            acc[:, pl.ds(i * TQ, TQ)] += _dot(_up(wo_s[...]), cb, NN)
            if i == FFN_UP:
                hh = ffn_up(h)
            if i > 0:
                projq((i - 1) * TQ)
            if i == FFN_DOWN:
                ffn_down(h, hh)
            projv(i * TQ)
            pp = pnext
        return carry

    lax.fori_loop(0, H - 1, head_step, 0)

    sel = sel_s[...]
    yT = y_s[...].T
    lane = lax.broadcasted_iota(jnp.int32, (1, 128), 1)
    for row in range(2):
        si = idx_s[row]
        r = _token_tile(si)
        upd = yT[:, row:row + 1] * sel[row:row + 1, 0:1]
        acc[:, r] += jnp.where(lane == (si & 127), upd, 0.0)

    def finish(i, cb):
        r = pl.ds(i * TQ, TQ)
        res = (1.0 - g_s[:, r]) * _up(xT[:, r]).astype(F32)
        obuf[:, r] = (acc[:, r] + res + _dot(_up(woT[H - 1]), cb, NN)).astype(BF)
        if i == OMID:
            o_copy(0, OMID + 1, 0).start()

    pp = scores(0, lone=True)
    pnext = scores(1)
    cb = context(0, pp)
    for i in range(1, NQ - 1):
        pp = pnext
        pnext = scores(i + 1, mid=functools.partial(finish, i - 1, cb))
        cb = context(i, pp)
    cb2 = context(NQ - 1, pnext, lone=True)
    finish(NQ - 2, cb)
    if O3:
        o_copy(OMID + 1, NQ - OMID - 2, 2).start()
    finish(NQ - 1, cb2)
    if O3:
        o_copy(NQ - 1, 1, 1).start()
        o_copy(OMID + 1, NQ - OMID - 2, 2).wait()
        o_copy(NQ - 1, 1, 1).wait()
    else:
        o_copy(OMID + 1, NQ - OMID - 1, 1).start()
        o_copy(OMID + 1, NQ - OMID - 1, 1).wait()
    o_copy(0, OMID + 1, 0).wait()


@jax.jit
def pallas_gated_mix__compressed_kv_cla__moe_arch_mod__prompt_kernel(
        A_x, A_c_kv, A_w_q, A_w_uk, A_w_uv, A_w_o, B_x, B_w_r, B_w_gate, B_w_up, B_w_down, gate_w):
    xT = jnp.transpose(A_x, (0, 2, 1)).reshape(M, S)
    c = A_c_kv.reshape(S, DC)
    woT = jnp.transpose(A_w_o, (0, 2, 1))
    wdT = B_w_down.T
    hbm = pl.BlockSpec(memory_space=pltpu.HBM)
    outT = pl.pallas_call(
        _kernel,
        in_specs=[hbm] * 11,
        out_specs=hbm,
        out_shape=jax.ShapeDtypeStruct((M, S), BF),
        scratch_shapes=[
            pltpu.VMEM((M // 2, S), U32),
            pltpu.VMEM((S // 2, DC), U32),
            pltpu.VMEM((2, M, D), U32),
            pltpu.VMEM((2, DC, D), U32),
            pltpu.VMEM((2, DC, D), U32),
            pltpu.VMEM((H, M // 2, D), U32),
            pltpu.VMEM((M // 2, F), U32),
            pltpu.VMEM((M // 2, F), U32),
            pltpu.VMEM((M // 2, F), U32),
            pltpu.VMEM((D // 2, M), U32),
            pltpu.VMEM((DC // 2, D), U32),
            pltpu.VMEM((D // 2, DC), U32),
            pltpu.VMEM((D // 2, S), U32),
            pltpu.VMEM((S // 2, D), U32),
            pltpu.VMEM((D // 2, S), U32),
            pltpu.VMEM((M, S), F32),
            pltpu.VMEM((M, S), BF),
            pltpu.VMEM((8, M), U32),
            pltpu.VMEM((16, M), F32),
            pltpu.VMEM((8, 128), F32),
            pltpu.VMEM((1, S), F32),
            pltpu.VMEM((8, M), U32),
            pltpu.VMEM((8, S), F32),
            pltpu.VMEM((M,), BF),
            pltpu.VMEM((M,), BF),
            pltpu.SMEM((2,), jnp.int32),
            pltpu.VMEM((M // 2, D), U32),
            pltpu.SemaphoreType.DMA((2, 3)),
            pltpu.SemaphoreType.DMA((NQ,)),
            pltpu.SemaphoreType.DMA((4,)),
            pltpu.SemaphoreType.DMA((10,)),
            pltpu.SemaphoreType.DMA((3,)),
        ],
        compiler_params=pltpu.CompilerParams(vmem_limit_bytes=100 * 1024 * 1024,
                                             disable_bounds_checks=True,
                                             disable_semaphore_checks=True),
        name="gated_mix",
    )(xT, c, A_w_q, A_w_uk, A_w_uv, woT, B_w_r, gate_w, B_w_gate, B_w_up, wdT)
    return jnp.transpose(outT.reshape(1, M, S), (0, 2, 1))
```

```python
import functools

import jax
import jax.numpy as jnp
from jax import lax
from jax.experimental import pallas as pl
from jax.experimental.pallas import tpu as pltpu

S = 2048
M = 448
DC = 1024
H = 16
D = 256
F = 1792
FT = 128
NF = F // FT
TQ = 256
NQ = S // TQ
XW = 512
FFN_UP, FFN_DOWN = 5, 3
OUT_FIRST = 6
LOG2E = 1.4426950408889634
QSCALE = (D ** -0.5) * LOG2E
NEG = -1e9 * LOG2E
BF = jnp.bfloat16
F32 = jnp.float32
U32 = jnp.uint32

NT = (((1,), (1,)), ((), ()))
NN = (((1,), (0,)), ((), ()))
_dot = functools.partial(lax.dot_general, preferred_element_type=F32)


def _pk(x):
    return pltpu.bitcast(x, U32)


def _up(x):
    return pltpu.bitcast(x, BF)


def _rows(start, n):
    return pl.ds(start // 2, n // 2)


def _token_tile(tok):
    t = jnp.clip(tok >> 7, 0, S // 128 - 1)
    return pl.ds(pl.multiple_of(t * 128, 128), 128)


def _head_of_pair(w32, parity):
    if isinstance(parity, int):
        bits = (w32 << 16) if parity == 0 else (w32 & jnp.uint32(0xFFFF0000))
    else:
        sh = (16 - 16 * parity).astype(U32)
        bits = lax.shift_left(w32, jnp.broadcast_to(sh, w32.shape)) & jnp.uint32(0xFFFF0000)
    return pltpu.bitcast(bits, F32)


def _split_dot(lhs_rows, n, parts, rhs):
    w = n // parts
    rr = [_dot(lhs_rows(w * u, w), rhs, NN) for u in range(parts)]
    return jnp.concatenate(rr, axis=0) if parts > 1 else rr[0]


def _kernel(xT_hbm, c_hbm, wq_hbm, wk_hbm, wv_hbm, woT_hbm, wr_hbm, gw_hbm,
            wg_hbm, wu_hbm, wdT_hbm, oT_hbm,
            xT, c, wq32, wk32, wv32, woT, wg, wu, wdT, wqT, wkb, wvT, qT, k_s, vT, acc, obuf,
            xsel, y_s, sel_s, g_s, rrows, rz_s, wr_ref, gw_ref, idx_s, wo_s,
            wsem, csem, xsem, msem, osem):

    def wq_copy(p, sl):
        return pltpu.make_async_copy(wq_hbm.bitcast(U32).at[:, p, :], wq32.at[sl], wsem.at[sl, 0])

    def wk_copy(p, sl):
        return pltpu.make_async_copy(wk_hbm.bitcast(U32).at[:, p, :], wk32.at[sl], wsem.at[sl, 1])

    def wv_copy(p, sl):
        return pltpu.make_async_copy(wv_hbm.bitcast(U32).at[:, p, :], wv32.at[sl], wsem.at[sl, 2])

    def c_copy(i):
        r = pl.ds(i * (TQ // 2), TQ // 2)
        return pltpu.make_async_copy(c_hbm.bitcast(U32).at[r, :], c.at[r, :], csem.at[i])

    def x_copy(i):
        r = pl.ds(i * XW, XW)
        return pltpu.make_async_copy(xT_hbm.bitcast(U32).at[:, r], xT.at[:, r], xsem.at[i])

    def side_copies(first):
        hs = pl.ds(0, 1) if first else pl.ds(1, H - 1)
        cs = pl.ds(0, FT) if first else pl.ds(FT, F - FT)
        o = 0 if first else 4
        return [pltpu.make_async_copy(woT_hbm.bitcast(U32).at[hs], woT.at[hs], msem.at[o]),
                pltpu.make_async_copy(wg_hbm.bitcast(U32).at[:, cs], wg.at[:, cs], msem.at[o + 1]),
                pltpu.make_async_copy(wu_hbm.bitcast(U32).at[:, cs], wu.at[:, cs], msem.at[o + 2]),
                pltpu.make_async_copy(wdT_hbm.bitcast(U32).at[:, cs], wdT.at[:, cs], msem.at[o + 3])]

    def vec_copies():
        return [pltpu.make_async_copy(wr_hbm, wr_ref, msem.at[8]),
                pltpu.make_async_copy(gw_hbm, gw_ref, msem.at[9])]

    def o_copy(i, n, k):
        r = pl.ds(i * TQ, n * TQ)
        return pltpu.make_async_copy(obuf.at[:, r], oT_hbm.at[:, r], osem.at[k])

    def prep_k(sl, parity):
        for r0 in range(0, DC, 128):
            wkb[_rows(r0, 128), :] = _pk(_head_of_pair(wk32[sl, pl.ds(r0, 128), :], parity).astype(BF))

    def prep_q(sl, parity):
        for r0 in range(0, M, 128):
            r = pl.ds(r0, min(128, M - r0))
            wqT[:, r] = _pk(_head_of_pair(wq32[sl, r, :], parity).T.astype(BF))

    def prep_v(sl, parity):
        for r0 in range(0, DC, 128):
            r = pl.ds(r0, 128)
            wvT[:, r] = _pk(_head_of_pair(wv32[sl, r, :], parity).T.astype(BF))

    def projk(pairs):
        k_s[pairs, :] = _pk(_dot(_up(c[pairs, :]), _up(wkb[...]), NN).astype(BF))

    def projv(toks, pairs):
        vT[:, toks] = _pk(_dot(_up(wvT[...]), _up(c[pairs, :]), NT).astype(BF))

    def projq(toks):
        qT[:, toks] = _pk((_dot(_up(wqT[...]), _up(xT[:, toks]), NN) * QSCALE).astype(BF))

    def scores(i, lone=False, mid=None):
        tri = (lax.broadcasted_iota(jnp.int32, (128, 128), 0)
               <= lax.broadcasted_iota(jnp.int32, (128, 128), 1))
        base = i * TQ
        nfull = base // 128
        chunks = []
        for j in range(nfull + 2):
            k0 = 128 * j
            if mid is not None and j == 2:
                mid()
            t0 = max(0, j - nfull)
            if j < nfull:
                if j % 2 == 0:
                    pair = _dot(_up(k_s[_rows(k0, 256), :]), _up(qT[:, pl.ds(base, TQ)]), NN)
                s = pair[128 * (j % 2):128 * (j % 2 + 1)]
            else:
                s = _split_dot(lambda a, n: _up(k_s[_rows(k0 + a, n), :]), 128,
                               2 if (lone and t0 == 1) else 1,
                               _up(qT[:, pl.ds(base + 128 * t0, TQ - 128 * t0)]))
                diag = jnp.where(tri, s[:, 0:128], NEG)
                s = jnp.concatenate([diag, s[:, 128:]], axis=1) if t0 == 0 else diag
            m = jnp.max(s, axis=0, keepdims=True)
            e = jnp.exp2(s - m)
            chunks.append((t0, m, jnp.sum(e, axis=0, keepdims=True), e.astype(BF)))
        return chunks

    def context(i, chunks, lone=False):
        scale = [[None, None] for _ in chunks]
        for t in range(2):
            js = [j for j, ch in enumerate(chunks) if ch[0] <= t]
            col = lambda x, j: x[:, 128 * (t - chunks[j][0]):128 * (t - chunks[j][0] + 1)]
            ms = [col(chunks[j][1], j) for j in js]
            m = functools.reduce(jnp.maximum, ms)
            al = [jnp.exp2(mj - m) for mj in ms]
            l = functools.reduce(jnp.add, [a * col(chunks[j][2], j) for a, j in zip(al, js)])
            li = g_s[:, pl.ds(i * TQ + 128 * t, 128)] / l
            for a, j in zip(al, js):
                scale[j][t] = a * li
        ctx = [None, None]
        n = len(chunks)
        for j in [n - 1, n - 2] + list(range(n - 2)):
            t0, _, _, p = chunks[j]
            parts = (4 if lone else 2) if j == n - 1 else (2 if j == n - 2 else 1)
            rr = _split_dot(lambda a, w: _up(vT[_rows(a, w), pl.ds(128 * j, 128)]), D, parts, p)
            for t in range(t0, 2):
                v = rr[:, 128 * (t - t0):128 * (t - t0 + 1)] * scale[j][t]
                ctx[t] = v if ctx[t] is None else ctx[t] + v
        return jnp.concatenate(ctx, axis=1).astype(BF)

    def router_rows():
        rows = lax.broadcasted_iota(jnp.int32, (16, M), 0)
        wr = jnp.broadcast_to(wr_ref[...].reshape(1, M).astype(F32), (16, M))
        gw = jnp.broadcast_to(gw_ref[...].reshape(1, M).astype(F32), (16, M))
        return jnp.where(rows == 0, wr, jnp.where(rows == 1, gw, 0.0)).astype(BF)

    def router():
        rz = rz_s[...]
        g = jax.nn.sigmoid(rz[1:2, :])
        g_s[...] = g
        rt = rz[0:1, :].astype(BF).astype(F32)
        tok = lax.broadcasted_iota(jnp.int32, (1, S), 1)
        m0 = jnp.max(rt, axis=1, keepdims=True)
        i0 = jnp.min(jnp.where(rt == m0, tok, S - 1), axis=1, keepdims=True)
        rt1 = jnp.where(tok == i0, -jnp.inf, rt)
        m1 = jnp.max(rt1, axis=1, keepdims=True)
        i1 = jnp.min(jnp.where((rt1 == m1) & (tok != i0), tok, S - 1), axis=1, keepdims=True)
        r16 = lax.broadcasted_iota(jnp.int32, (16, 128), 0)
        l16 = lax.broadcasted_iota(jnp.int32, (16, 128), 1)
        xs = None
        wsel = []
        for row, idx, mx in ((0, i0, m0), (1, i1, m1)):
            si = jnp.max(idx)
            idx_s[row] = si
            tile = _up(xT[:, _token_tile(si)])
            onehot = jnp.where((r16 == row) & (l16 == (idx & 127)), 1.0, 0.0).astype(BF)
            part = _dot(onehot, tile, NT)
            xs = part if xs is None else xs + part
            keep = jnp.sum(jnp.where(tok == idx, 1.0 - g, 0.0), axis=1, keepdims=True)
            wsel.append(jnp.broadcast_to(jax.nn.sigmoid(mx) * keep, (8, 128)))
        xsel[...] = _pk(xs.astype(BF))
        r8 = lax.broadcasted_iota(jnp.int32, (8, 128), 0)
        sel_s[...] = jnp.where(r8 == 0, wsel[0], wsel[1])
        y_s[...] = jnp.zeros_like(y_s)

    def ffn_cols(h):
        return pl.ds(pl.multiple_of(jnp.minimum(h, NF - 1) * FT, FT), FT)

    def ffn_up(h):
        xs = _up(xsel[...])
        gg = _dot(xs, _up(wg[:, ffn_cols(h)]), NN)
        uu = _dot(xs, _up(wu[:, ffn_cols(h)]), NN)
        return (gg * jax.nn.sigmoid(gg) * uu).astype(BF)

    def ffn_down(h, hh):
        y_s[...] += jnp.where(h < NF, _dot(hh, _up(wdT[:, ffn_cols(h)]), NT), 0.0)

    wq_copy(0, 0).start()
    for cp in vec_copies():
        cp.start()
    for i in range(S // XW):
        x_copy(i).start()
    wk_copy(0, 0).start()
    for i in range(NQ):
        c_copy(i).start()
        if i == 1:
            wv_copy(0, 0).start()
    for cp in side_copies(True):
        cp.start()
    wq_copy(1, 1).start()
    wk_copy(1, 1).start()
    wv_copy(1, 1).start()
    for cp in side_copies(False):
        cp.start()
    acc[...] = jnp.zeros_like(acc)

    wq_copy(0, 0).wait()
    for cp in vec_copies():
        cp.wait()
    rrows[...] = _pk(router_rows())
    prep_q(0, 0)

    def q_first(i, carry):
        x_copy(i).wait()
        r = pl.ds(pl.multiple_of(i * XW, XW), XW)
        lhs = jnp.concatenate([_up(wqT[...]), _up(rrows[...])], axis=0)
        res = _dot(lhs, _up(xT[:, r]), NN)
        qT[:, r] = _pk((res[:D] * QSCALE).astype(BF))
        rz_s[:, r] = res[D:D + 8]
        return carry
    lax.fori_loop(0, S // XW, q_first, 0)

    wk_copy(0, 0).wait()
    prep_k(0, 0)

    def k_first(i, carry):
        c_copy(i).wait()
        projk(pl.ds(pl.multiple_of(i * (TQ // 2), TQ // 2), TQ // 2))
        return carry
    lax.fori_loop(0, XW // TQ, k_first, 0)

    wv_copy(0, 0).wait()
    prep_v(0, 0)
    projv(pl.ds(0, XW), _rows(0, XW))
    router()

    def kv_first(i, carry):
        c_copy(2 * i).wait()
        c_copy(2 * i + 1).wait()
        pairs = pl.ds(pl.multiple_of(i * (XW // 2), XW // 2), XW // 2)
        projk(pairs)
        projv(pl.ds(pl.multiple_of(i * XW, XW), XW), pairs)
        return carry
    lax.fori_loop(1, S // XW, kv_first, 0)
    for cp in side_copies(True):
        cp.wait()

    def head_step(h, carry):
        pn = (h + 1) >> 1

        @pl.when((h & 1) == 1)
        def _():
            wq_copy(pn, pn & 1).wait()
            wk_copy(pn, pn & 1).wait()
            wv_copy(pn, pn & 1).wait()

            @pl.when(pn + 1 < H // 2)
            def _():
                wq_copy(pn + 1, 1 - (pn & 1)).start()
                wk_copy(pn + 1, 1 - (pn & 1)).start()
                wv_copy(pn + 1, 1 - (pn & 1)).start()

            @pl.when(h == 1)
            def _():
                for cp in side_copies(False):
                    cp.wait()

        prep_k(pn & 1, (h + 1) & 1)
        prep_q(pn & 1, (h + 1) & 1)
        prep_v(pn & 1, (h + 1) & 1)
        wo_s[...] = woT[h]
        cur = scores(NQ - 1, lone=True)
        projq(pl.ds((NQ - 1) * TQ, TQ))
        for i in range(NQ - 1, -1, -1):
            nxt = scores(i - 1) if i > 0 else None
            cb = context(i, cur, lone=(i == 0))
            projv(pl.ds(i * TQ, TQ), _rows(i * TQ, TQ))
            projk(_rows(i * TQ, TQ))
            acc[:, pl.ds(i * TQ, TQ)] += _dot(_up(wo_s[...]), cb, NN)
            if i == FFN_UP:
                hh = ffn_up(h)
            if i > 0:
                projq(pl.ds((i - 1) * TQ, TQ))
            if i == FFN_DOWN:
                ffn_down(h, hh)
            cur = nxt
        return carry

    lax.fori_loop(0, H - 1, head_step, 0)

    sel = sel_s[...]
    yT = y_s[...].T
    lane = lax.broadcasted_iota(jnp.int32, (1, 128), 1)
    for row in range(2):
        si = idx_s[row]
        r = _token_tile(si)
        upd = yT[:, row:row + 1] * sel[row:row + 1, 0:1]
        acc[:, r] += jnp.where(lane == (si & 127), upd, 0.0)

    outs = [o_copy(0, OUT_FIRST, 0), o_copy(OUT_FIRST, NQ - 1 - OUT_FIRST, 1), o_copy(NQ - 1, 1, 2)]

    def finish(i, cb):
        r = pl.ds(i * TQ, TQ)
        res = (1.0 - g_s[:, r]) * _up(xT[:, r]).astype(F32)
        obuf[:, r] = (acc[:, r] + res + _dot(_up(woT[H - 1]), cb, NN)).astype(BF)
        if i == OUT_FIRST - 1:
            outs[0].start()

    cur = scores(0, lone=True)
    nxt = scores(1)
    cb = context(0, cur)
    for i in range(1, NQ - 1):
        cur = nxt
        nxt = scores(i + 1, mid=functools.partial(finish, i - 1, cb))
        cb = context(i, cur)
    cb_last = context(NQ - 1, nxt, lone=True)
    finish(NQ - 2, cb)
    outs[1].start()
    finish(NQ - 1, cb_last)
    outs[2].start()
    for cp in outs:
        cp.wait()


@jax.jit
def pallas_gated_mix__compressed_kv_cla__moe_arch_mod__prompt_kernel(
        A_x, A_c_kv, A_w_q, A_w_uk, A_w_uv, A_w_o, B_x, B_w_r, B_w_gate, B_w_up, B_w_down, gate_w):
    xT = jnp.transpose(A_x, (0, 2, 1)).reshape(M, S)
    c = A_c_kv.reshape(S, DC)
    woT = jnp.transpose(A_w_o, (0, 2, 1))
    wdT = B_w_down.T
    hbm = pl.BlockSpec(memory_space=pltpu.HBM)
    outT = pl.pallas_call(
        _kernel,
        in_specs=[hbm] * 11,
        out_specs=hbm,
        out_shape=jax.ShapeDtypeStruct((M, S), BF),
        scratch_shapes=[
            pltpu.VMEM((M // 2, S), U32),
            pltpu.VMEM((S // 2, DC), U32),
            pltpu.VMEM((2, M, D), U32),
            pltpu.VMEM((2, DC, D), U32),
            pltpu.VMEM((2, DC, D), U32),
            pltpu.VMEM((H, M // 2, D), U32),
            pltpu.VMEM((M // 2, F), U32),
            pltpu.VMEM((M // 2, F), U32),
            pltpu.VMEM((M // 2, F), U32),
            pltpu.VMEM((D // 2, M), U32),
            pltpu.VMEM((DC // 2, D), U32),
            pltpu.VMEM((D // 2, DC), U32),
            pltpu.VMEM((D // 2, S), U32),
            pltpu.VMEM((S // 2, D), U32),
            pltpu.VMEM((D // 2, S), U32),
            pltpu.VMEM((M, S), F32),
            pltpu.VMEM((M, S), BF),
            pltpu.VMEM((8, M), U32),
            pltpu.VMEM((16, M), F32),
            pltpu.VMEM((8, 128), F32),
            pltpu.VMEM((1, S), F32),
            pltpu.VMEM((8, M), U32),
            pltpu.VMEM((8, S), F32),
            pltpu.VMEM((M,), BF),
            pltpu.VMEM((M,), BF),
            pltpu.SMEM((2,), jnp.int32),
            pltpu.VMEM((M // 2, D), U32),
            pltpu.SemaphoreType.DMA((2, 3)),
            pltpu.SemaphoreType.DMA((NQ,)),
            pltpu.SemaphoreType.DMA((S // XW,)),
            pltpu.SemaphoreType.DMA((10,)),
            pltpu.SemaphoreType.DMA((3,)),
        ],
        compiler_params=pltpu.CompilerParams(vmem_limit_bytes=100 * 1024 * 1024,
                                             disable_bounds_checks=True,
                                             disable_semaphore_checks=True),
        name="gated_mix",
    )(xT, c, A_w_q, A_w_uk, A_w_uv, woT, B_w_r, gate_w, B_w_gate, B_w_up, wdT)
    return jnp.transpose(outT.reshape(1, M, S), (0, 2, 1))
```

```python
import functools

import jax
import jax.numpy as jnp
from jax import lax
from jax.experimental import pallas as pl
from jax.experimental.pallas import tpu as pltpu

S = 2048
M = 448
DC = 1024
H = 16
D = 256
F = 1792
FT = 128
NF = F // FT
TQ = 256
NQ = S // TQ
XW = 512
FFN_UP, FFN_DOWN = 5, 3
FETCH_AT = 4
LOG2E = 1.4426950408889634
QSCALE = (D ** -0.5) * LOG2E
NEG = -1e9 * LOG2E
BF = jnp.bfloat16
F32 = jnp.float32
U32 = jnp.uint32

NT = (((1,), (1,)), ((), ()))
NN = (((1,), (0,)), ((), ()))
_dot = functools.partial(lax.dot_general, preferred_element_type=F32)


def _pk(x):
    return pltpu.bitcast(x, U32)


def _up(x):
    return pltpu.bitcast(x, BF)


def _rows(start, n):
    return pl.ds(start // 2, n // 2)


def _token_tile(tok):
    t = jnp.clip(tok >> 7, 0, S // 128 - 1)
    return pl.ds(pl.multiple_of(t * 128, 128), 128)


def _head_of_pair(w32, parity):
    if isinstance(parity, int):
        bits = (w32 << 16) if parity == 0 else (w32 & jnp.uint32(0xFFFF0000))
    else:
        sh = (16 - 16 * parity).astype(U32)
        bits = lax.shift_left(w32, jnp.broadcast_to(sh, w32.shape)) & jnp.uint32(0xFFFF0000)
    return pltpu.bitcast(bits, F32)


def _split_dot(lhs_rows, n, parts, rhs):
    w = n // parts
    rr = [_dot(lhs_rows(w * u, w), rhs, NN) for u in range(parts)]
    return jnp.concatenate(rr, axis=0) if parts > 1 else rr[0]


def _kernel(xT_hbm, c_hbm, wq_hbm, wk_hbm, wv_hbm, woT_hbm, wr_hbm, gw_hbm,
            wg_hbm, wu_hbm, wdT_hbm, oT_hbm,
            xT, c, raw, woT, wg, wu, wdT, wqT, wkb, wvT, qT, k_s, vT, acc, obuf,
            xsel, y_s, sel_s, g_s, rrows, rz_s, wr_ref, gw_ref, idx_s, wo_s,
            wsem, csem, xsem, msem, osem):

    def w_copies(which, p, sem):
        w_hbm, r0, n = ((wq_hbm, 0, M), (wk_hbm, M, DC), (wv_hbm, M + DC, DC))[which]
        return [pltpu.make_async_copy(w_hbm.bitcast(U32).at[:, p, pl.ds(128 * t, 128)],
                                      raw.at[t, pl.ds(r0, n), :], wsem.at[sem]) for t in range(D // 128)]

    def pair_copies(p):
        return [cp for which in range(3) for cp in w_copies(which, p, 3)]

    def raw_rows(r0, n):
        return jnp.concatenate([raw[t, pl.ds(r0, n), :] for t in range(D // 128)], axis=1)

    def c_copy(i):
        r = pl.ds(i * (TQ // 2), TQ // 2)
        return pltpu.make_async_copy(c_hbm.bitcast(U32).at[r, :], c.at[r, :], csem.at[i])

    def x_copy(i):
        r = pl.ds(i * XW, XW)
        return pltpu.make_async_copy(xT_hbm.bitcast(U32).at[:, r], xT.at[:, r], xsem.at[i])

    def side_copies(first):
        hs = pl.ds(0, 1) if first else pl.ds(1, H - 1)
        cs = pl.ds(0, FT) if first else pl.ds(FT, F - FT)
        sem = msem.at[0 if first else 1]
        return [pltpu.make_async_copy(woT_hbm.bitcast(U32).at[hs], woT.at[hs], sem),
                pltpu.make_async_copy(wg_hbm.bitcast(U32).at[:, cs], wg.at[:, cs], sem),
                pltpu.make_async_copy(wu_hbm.bitcast(U32).at[:, cs], wu.at[:, cs], sem),
                pltpu.make_async_copy(wdT_hbm.bitcast(U32).at[:, cs], wdT.at[:, cs], sem)]

    def vec_copies():
        return [pltpu.make_async_copy(wr_hbm, wr_ref, msem.at[2]),
                pltpu.make_async_copy(gw_hbm, gw_ref, msem.at[3])]

    def prep_k(parity):
        for r0 in range(0, DC, 128):
            wkb[_rows(r0, 128), :] = _pk(_head_of_pair(raw_rows(M + r0, 128), parity).astype(BF))

    def prep_q(parity):
        for r0 in range(0, M, 128):
            n = min(128, M - r0)
            wqT[:, pl.ds(r0, n)] = _pk(_head_of_pair(raw_rows(r0, n), parity).T.astype(BF))

    def prep_v(parity):
        for r0 in range(0, DC, 128):
            wvT[:, pl.ds(r0, 128)] = _pk(_head_of_pair(raw_rows(M + DC + r0, 128), parity).T.astype(BF))

    def projk(pairs):
        k_s[pairs, :] = _pk(_dot(_up(c[pairs, :]), _up(wkb[...]), NN).astype(BF))

    def projv(toks, pairs):
        vT[:, toks] = _pk(_dot(_up(wvT[...]), _up(c[pairs, :]), NT).astype(BF))

    def projq(toks):
        qT[:, toks] = _pk((_dot(_up(wqT[...]), _up(xT[:, toks]), NN) * QSCALE).astype(BF))

    def scores(i, lone=False, mid=None):
        tri = (lax.broadcasted_iota(jnp.int32, (128, 128), 0)
               <= lax.broadcasted_iota(jnp.int32, (128, 128), 1))
        base = i * TQ
        nfull = base // 128
        chunks = []
        for j in range(nfull + 2):
            k0 = 128 * j
            if mid is not None and j == 2:
                mid()
            t0 = max(0, j - nfull)
            if j < nfull:
                if j % 2 == 0:
                    pair = _dot(_up(k_s[_rows(k0, 256), :]), _up(qT[:, pl.ds(base, TQ)]), NN)
                s = pair[128 * (j % 2):128 * (j % 2 + 1)]
            else:
                s = _split_dot(lambda a, n: _up(k_s[_rows(k0 + a, n), :]), 128,
                               2 if (lone and t0 == 1) else 1,
                               _up(qT[:, pl.ds(base + 128 * t0, TQ - 128 * t0)]))
                diag = jnp.where(tri, s[:, 0:128], NEG)
                s = jnp.concatenate([diag, s[:, 128:]], axis=1) if t0 == 0 else diag
            m = jnp.max(s, axis=0, keepdims=True)
            e = jnp.exp2(s - m)
            chunks.append((t0, m, jnp.sum(e, axis=0, keepdims=True), e.astype(BF)))
        return chunks

    def context(i, chunks, lone=False):
        scale = [[None, None] for _ in chunks]
        for t in range(2):
            js = [j for j, ch in enumerate(chunks) if ch[0] <= t]
            col = lambda x, j: x[:, 128 * (t - chunks[j][0]):128 * (t - chunks[j][0] + 1)]
            ms = [col(chunks[j][1], j) for j in js]
            m = functools.reduce(jnp.maximum, ms)
            al = [jnp.exp2(mj - m) for mj in ms]
            l = functools.reduce(jnp.add, [a * col(chunks[j][2], j) for a, j in zip(al, js)])
            li = g_s[:, pl.ds(i * TQ + 128 * t, 128)] / l
            for a, j in zip(al, js):
                scale[j][t] = a * li
        ctx = [None, None]
        n = len(chunks)
        for j in [n - 1, n - 2] + list(range(n - 2)):
            t0, _, _, p = chunks[j]
            parts = (4 if lone else 2) if j == n - 1 else (2 if j == n - 2 else 1)
            rr = _split_dot(lambda a, w: _up(vT[_rows(a, w), pl.ds(128 * j, 128)]), D, parts, p)
            for t in range(t0, 2):
                v = rr[:, 128 * (t - t0):128 * (t - t0 + 1)] * scale[j][t]
                ctx[t] = v if ctx[t] is None else ctx[t] + v
        return jnp.concatenate(ctx, axis=1).astype(BF)

    def router_rows():
        rows = lax.broadcasted_iota(jnp.int32, (16, M), 0)
        wr = jnp.broadcast_to(wr_ref[...].reshape(1, M).astype(F32), (16, M))
        gw = jnp.broadcast_to(gw_ref[...].reshape(1, M).astype(F32), (16, M))
        return jnp.where(rows == 0, wr, jnp.where(rows == 1, gw, 0.0)).astype(BF)

    def router():
        rz = rz_s[...]
        g = jax.nn.sigmoid(rz[1:2, :])
        g_s[...] = g
        rt = rz[0:1, :].astype(BF).astype(F32)
        tok = lax.broadcasted_iota(jnp.int32, (1, S), 1)
        m0 = jnp.max(rt, axis=1, keepdims=True)
        i0 = jnp.min(jnp.where(rt == m0, tok, S - 1), axis=1, keepdims=True)
        rt1 = jnp.where(tok == i0, -jnp.inf, rt)
        m1 = jnp.max(rt1, axis=1, keepdims=True)
        i1 = jnp.min(jnp.where((rt1 == m1) & (tok != i0), tok, S - 1), axis=1, keepdims=True)
        r16 = lax.broadcasted_iota(jnp.int32, (16, 128), 0)
        l16 = lax.broadcasted_iota(jnp.int32, (16, 128), 1)
        xs = None
        wsel = []
        for row, idx, mx in ((0, i0, m0), (1, i1, m1)):
            si = jnp.max(idx)
            idx_s[row] = si
            tile = _up(xT[:, _token_tile(si)])
            onehot = jnp.where((r16 == row) & (l16 == (idx & 127)), 1.0, 0.0).astype(BF)
            part = _dot(onehot, tile, NT)
            xs = part if xs is None else xs + part
            keep = jnp.sum(jnp.where(tok == idx, 1.0 - g, 0.0), axis=1, keepdims=True)
            wsel.append(jnp.broadcast_to(jax.nn.sigmoid(mx) * keep, (8, 128)))
        xsel[...] = _pk(xs.astype(BF))
        r8 = lax.broadcasted_iota(jnp.int32, (8, 128), 0)
        sel_s[...] = jnp.where(r8 == 0, wsel[0], wsel[1])
        y_s[...] = jnp.zeros_like(y_s)

    def ffn_cols(h):
        return pl.ds(pl.multiple_of(jnp.minimum(h, NF - 1) * FT, FT), FT)

    def ffn_up(h):
        xs = _up(xsel[...])
        gg = _dot(xs, _up(wg[:, ffn_cols(h)]), NN)
        uu = _dot(xs, _up(wu[:, ffn_cols(h)]), NN)
        return (gg * jax.nn.sigmoid(gg) * uu).astype(BF)

    def ffn_down(h, hh):
        y_s[...] += jnp.where(h < NF, _dot(hh, _up(wdT[:, ffn_cols(h)]), NT), 0.0)

    wq0, wk0, wv0 = (w_copies(which, 0, which) for which in range(3))
    for cp in wq0 + vec_copies():
        cp.start()
    for i in range(S // XW):
        x_copy(i).start()
    for cp in wk0:
        cp.start()
    for i in range(NQ):
        c_copy(i).start()
        if i == 1:
            for cp in wv0:
                cp.start()
    for cp in side_copies(True):
        cp.start()
    for cp in side_copies(False):
        cp.start()
    acc[...] = jnp.zeros_like(acc)

    for cp in wq0 + vec_copies():
        cp.wait()
    rrows[...] = _pk(router_rows())
    prep_q(0)

    def q_first(i, carry):
        x_copy(i).wait()
        r = pl.ds(pl.multiple_of(i * XW, XW), XW)
        lhs = jnp.concatenate([_up(wqT[...]), _up(rrows[...])], axis=0)
        res = _dot(lhs, _up(xT[:, r]), NN)
        qT[:, r] = _pk((res[:D] * QSCALE).astype(BF))
        rz_s[:, r] = res[D:D + 8]
        return carry
    lax.fori_loop(0, S // XW, q_first, 0)

    for cp in wk0:
        cp.wait()
    prep_k(0)

    def k_first(i, carry):
        c_copy(i).wait()
        projk(pl.ds(pl.multiple_of(i * (TQ // 2), TQ // 2), TQ // 2))
        return carry
    lax.fori_loop(0, XW // TQ, k_first, 0)

    for cp in wv0:
        cp.wait()
    prep_v(0)
    projv(pl.ds(0, XW), _rows(0, XW))
    router()

    def kv_first(i, carry):
        c_copy(2 * i).wait()
        c_copy(2 * i + 1).wait()
        pairs = pl.ds(pl.multiple_of(i * (XW // 2), XW // 2), XW // 2)
        projk(pairs)
        projv(pl.ds(pl.multiple_of(i * XW, XW), XW), pairs)
        return carry
    lax.fori_loop(1, S // XW, kv_first, 0)
    for cp in side_copies(True):
        cp.wait()

    def head_step(h, carry):
        pn = (h + 1) >> 1

        @pl.when((h & 1) == 1)
        def _():
            for cp in pair_copies(pn):
                cp.wait()

        @pl.when(h == 1)
        def _():
            for cp in side_copies(False):
                cp.wait()

        prep_k((h + 1) & 1)
        prep_q((h + 1) & 1)
        prep_v((h + 1) & 1)
        wo_s[...] = woT[h]
        cur = scores(NQ - 1, lone=True)
        projq(pl.ds((NQ - 1) * TQ, TQ))
        for i in range(NQ - 1, -1, -1):
            nxt = scores(i - 1) if i > 0 else None
            cb = context(i, cur, lone=(i == 0))
            projv(pl.ds(i * TQ, TQ), _rows(i * TQ, TQ))
            projk(_rows(i * TQ, TQ))
            acc[:, pl.ds(i * TQ, TQ)] += _dot(_up(wo_s[...]), cb, NN)
            if i == FFN_UP:
                hh = ffn_up(h)
            if i > 0:
                projq(pl.ds((i - 1) * TQ, TQ))
            if i == FFN_DOWN:
                ffn_down(h, hh)
            if i == FETCH_AT:
                @pl.when(jnp.logical_and((h & 1) == 0, pn + 1 < H // 2))
                def _():
                    for cp in pair_copies(pn + 1):
                        cp.start()
            cur = nxt
        return carry

    lax.fori_loop(0, H - 1, head_step, 0)

    sel = sel_s[...]
    yT = y_s[...].T
    lane = lax.broadcasted_iota(jnp.int32, (1, 128), 1)
    for row in range(2):
        si = idx_s[row]
        r = _token_tile(si)
        upd = yT[:, row:row + 1] * sel[row:row + 1, 0:1]
        acc[:, r] += jnp.where(lane == (si & 127), upd, 0.0)

    outs = []

    def finish(i, cb):
        r = pl.ds(i * TQ, TQ)
        res = (1.0 - g_s[:, r]) * _up(xT[:, r]).astype(F32)
        obuf[:, r] = (acc[:, r] + res + _dot(_up(woT[H - 1]), cb, NN)).astype(BF)
        outs.append(pltpu.make_async_copy(obuf.at[:, r], oT_hbm.at[:, r], osem.at[0]))
        outs[-1].start()

    cur = scores(0, lone=True)
    nxt = scores(1)
    cb = context(0, cur)
    for i in range(1, NQ - 1):
        cur = nxt
        nxt = scores(i + 1, mid=functools.partial(finish, i - 1, cb))
        cb = context(i, cur)
    cb_last = context(NQ - 1, nxt, lone=True)
    finish(NQ - 2, cb)
    finish(NQ - 1, cb_last)
    for cp in outs:
        cp.wait()


@jax.jit
def pallas_gated_mix__compressed_kv_cla__moe_arch_mod__prompt_kernel(
        A_x, A_c_kv, A_w_q, A_w_uk, A_w_uv, A_w_o, B_x, B_w_r, B_w_gate, B_w_up, B_w_down, gate_w):
    xT = jnp.transpose(A_x, (0, 2, 1)).reshape(M, S)
    c = A_c_kv.reshape(S, DC)
    woT = jnp.transpose(A_w_o, (0, 2, 1))
    wdT = B_w_down.T
    hbm = pl.BlockSpec(memory_space=pltpu.HBM)
    outT = pl.pallas_call(
        _kernel,
        in_specs=[hbm] * 11,
        out_specs=hbm,
        out_shape=jax.ShapeDtypeStruct((M, S), BF),
        scratch_shapes=[
            pltpu.VMEM((M // 2, S), U32),
            pltpu.VMEM((S // 2, DC), U32),
            pltpu.VMEM((D // 128, M + 2 * DC, 128), U32),
            pltpu.VMEM((H, M // 2, D), U32),
            pltpu.VMEM((M // 2, F), U32),
            pltpu.VMEM((M // 2, F), U32),
            pltpu.VMEM((M // 2, F), U32),
            pltpu.VMEM((D // 2, M), U32),
            pltpu.VMEM((DC // 2, D), U32),
            pltpu.VMEM((D // 2, DC), U32),
            pltpu.VMEM((D // 2, S), U32),
            pltpu.VMEM((S // 2, D), U32),
            pltpu.VMEM((D // 2, S), U32),
            pltpu.VMEM((M, S), F32),
            pltpu.VMEM((M, S), BF),
            pltpu.VMEM((8, M), U32),
            pltpu.VMEM((16, M), F32),
            pltpu.VMEM((8, 128), F32),
            pltpu.VMEM((1, S), F32),
            pltpu.VMEM((8, M), U32),
            pltpu.VMEM((8, S), F32),
            pltpu.VMEM((M,), BF),
            pltpu.VMEM((M,), BF),
            pltpu.SMEM((2,), jnp.int32),
            pltpu.VMEM((M // 2, D), U32),
            pltpu.SemaphoreType.DMA((4,)),
            pltpu.SemaphoreType.DMA((NQ,)),
            pltpu.SemaphoreType.DMA((S // XW,)),
            pltpu.SemaphoreType.DMA((4,)),
            pltpu.SemaphoreType.DMA((1,)),
        ],
        compiler_params=pltpu.CompilerParams(vmem_limit_bytes=100 * 1024 * 1024,
                                             disable_bounds_checks=True,
                                             disable_semaphore_checks=True),
        name="gated_mix",
    )(xT, c, A_w_q, A_w_uk, A_w_uv, woT, B_w_r, gate_w, B_w_gate, B_w_up, wdT)
    return jnp.transpose(outT.reshape(1, M, S), (0, 2, 1))
```
